```python
import jax
import jax.numpy as jnp

def _softmax(x, axis=-1):
    return jax.nn.softmax(x, axis=axis)
def _gelu(x):
    return jax.nn.gelu(x, approximate=True)
def _silu(x):
    return jax.nn.silu(x)
def _sigmoid(x):
    return jax.nn.sigmoid(x)
def _layernorm(x, axis=-1, eps=1e-5):
    m = jnp.mean(x, axis=axis, keepdims=True)
    v = jnp.var(x, axis=axis, keepdims=True)
    return (x - m) / jnp.sqrt(v + eps)
def _scatter_add(tgt, idx, src, axis=0):
    return tgt.at[idx].add(src)
def _segment_sum(src, seg, n):
    return jax.ops.segment_sum(src, seg, n)
class _Rng:
    def __init__(self, key):
        self._k = key
    def _next(self):
        self._k, sub = jax.random.split(self._k)
        return sub
    def normal(self, shape):
        return jax.random.normal(self._next(), shape, dtype=jnp.bfloat16)
    def randint(self, lo, hi, shape):
        return jax.random.randint(self._next(), shape, lo, hi, dtype=jnp.int32)
    def uniform(self, shape, lo=0.0, hi=1.0):
        return jax.random.uniform(self._next(), shape, jnp.bfloat16, lo, hi)
    def permutation(self, n):
        return jax.random.permutation(self._next(), n)


kernel_name = 'standalone__fused_io_aware_attn__prompt'

def setup_inputs():
    _rng = _Rng(jax.random.key(int.from_bytes(__import__("os").urandom(4), "little")))
    _w = (lambda a: (lambda t: t.astype(jnp.bfloat16) if jnp.issubdtype(t.dtype, jnp.floating) else t)(jnp.asarray(a)))
    B, H, S = 2, 32, 2048
    Dh = max(1, 1024 // 32)
    return {
        "q": _w((lambda *s: _rng.normal(s) * 0.05)(B, H, S, Dh)),
        "k": _w((lambda *s: _rng.normal(s) * 0.05)(B, H, S, Dh)),
        "v": _w((lambda *s: _rng.normal(s) * 0.05)(B, H, S, Dh)),
    }

def reference(q, k, v):
    scale = q.shape[-1] ** -0.5
    s = jnp.einsum('bhqd,bhkd->bhqk', q, k) * scale
    p = _softmax(s, axis=-1)
    return jnp.einsum('bhqk,bhkd->bhqd', p, v)
```

```python
import functools, math
import jax, jax.numpy as jnp, numpy as np
from jax import lax
from jax.experimental import pallas as pl
from jax.experimental.pallas import tpu as pltpu

LOG2E = 1.4426950408889634

def make(BQ=512, CK=128, SUB=128, vmem=100*2**20, flags=None, accmem=True, tn=False, unroll=1, lmode=0):
    def kernel(qT_ref, kT_ref, vT_ref, oT_ref, k_scr, s_scr, m_scr, o_scr, l_scr, *, NH):
        D = qT_ref.shape[0]
        S = kT_ref.shape[1]
        c = (D ** -0.5) * LOG2E
        t = pl.program_id(0)

        if not tn:
            @pl.when(t < NH)
            def _():
                k_scr[...] = kT_ref[...].astype(jnp.float32).T.astype(jnp.bfloat16)

        def body(j, do_a, do_b):
            cs = pl.ds(pl.multiple_of(j * BQ, BQ), BQ)
            if do_a:
                qT = (qT_ref[:, cs].astype(jnp.float32) * c).astype(jnp.bfloat16)
            if do_b:
                m_prev = m_scr[:, cs]
            mx = None
            l = None
            o = None
            for ck in range(S // CK):
                ps = []
                lc = None
                for sb in range(CK // SUB):
                    r0 = ck * CK + sb * SUB
                    if do_b:
                        p = jnp.exp2(s_scr[r0:r0+SUB, cs] - m_prev)
                        ls = jnp.sum(p.reshape(SUB // 8, 8, BQ), axis=0)
                        lc = ls if lc is None else lc + ls
                        ps.append(p.astype(jnp.bfloat16))
                    if do_a:
                        if tn:
                            sT = lax.dot_general(kT_ref[:, r0:r0+SUB], qT, (((0,), (0,)), ((), ())), preferred_element_type=jnp.float32)
                        else:
                            sT = jnp.dot(k_scr[r0:r0+SUB, :], qT, preferred_element_type=jnp.float32)
                        s_scr[r0:r0+SUB, cs] = sT
                        mm = jnp.max(sT.reshape(SUB // 8, 8, BQ), axis=0)
                        mx = mm if mx is None else jnp.maximum(mx, mm)
                if do_b:
                    p = ps[0] if len(ps) == 1 else jnp.concatenate(ps, axis=0)
                    ob = jnp.dot(vT_ref[:, ck*CK:(ck+1)*CK], p, preferred_element_type=jnp.float32)
                    if accmem:
                        if ck == 0:
                            o_scr[...] = ob
                            l_scr[...] = lc
                        else:
                            o_scr[...] += ob
                            l_scr[...] += lc
                    else:
                        o = ob if o is None else o + ob
                        l = lc if l is None else l + lc
            if do_a:
                m_scr[:, cs] = jnp.max(mx, axis=0, keepdims=True)
            if do_b:
                if accmem:
                    o = o_scr[...]; l = l_scr[...]
                lt = jnp.sum(l, axis=0, keepdims=True)
                oT_ref[:, cs] = (o / lt).astype(oT_ref.dtype)

        def loop(do_a, do_b):
            def f(j, carry):
                body(j, do_a, do_b)
                return carry
            lax.fori_loop(0, S // BQ, f, 0, unroll=unroll if (do_a and do_b) else 1)

        @pl.when(t == 0)
        def _():
            loop(True, False)
        @pl.when((t > 0) & (t < NH))
        def _():
            loop(True, True)
        @pl.when(t == NH)
        def _():
            loop(False, True)

    def fn(q, k, v):
        B, H, S, D = q.shape
        NH = B * H
        qT = jnp.swapaxes(q, 2, 3).reshape(NH, D, S)
        kT = jnp.swapaxes(k, 2, 3).reshape(NH, D, S)
        vT = jnp.swapaxes(v, 2, 3).reshape(NH, D, S)
        def cur(t): return jnp.minimum(t, NH - 1)
        def prv(t): return jnp.maximum(t - 1, 0)
        oT = pl.pallas_call(
            functools.partial(kernel, NH=NH),
            grid=(NH + 1,),
            in_specs=[
                pl.BlockSpec((None, D, S), lambda t: (cur(t), 0, 0)),
                pl.BlockSpec((None, D, S), lambda t: (cur(t), 0, 0)),
                pl.BlockSpec((None, D, S), lambda t: (prv(t), 0, 0)),
            ],
            out_specs=pl.BlockSpec((None, D, S), lambda t: (prv(t), 0, 0)),
            out_shape=jax.ShapeDtypeStruct((NH, D, S), q.dtype),
            scratch_shapes=[pltpu.VMEM((S, D), jnp.bfloat16), pltpu.VMEM((S, S), jnp.float32), pltpu.VMEM((1, S), jnp.float32),
                            pltpu.VMEM((D, BQ), jnp.float32), pltpu.VMEM((8, BQ), jnp.float32)],
            compiler_params=pltpu.CompilerParams(
                dimension_semantics=("arbitrary",), vmem_limit_bytes=vmem,
                **({"flags": flags} if flags else {})),
            name="attn",
        )(qT, kT, vT)
        return jnp.swapaxes(oT.reshape(B, H, D, S), 2, 3)
    return fn


_impl = make(**dict())


@jax.jit
def pallas_standalone__fused_io_aware_attn__prompt_kernel(q, k, v):
    return _impl(q, k, v)
```

```python
import functools
import jax, jax.numpy as jnp
from jax import lax
from jax.experimental import pallas as pl
from jax.experimental.pallas import tpu as pltpu

LOG2E = 1.4426950408889634


def _body(q_ref, k_ref, v_ref, o_ref, s_scr, m_scr, o_scr, l_scr, *, do_a, do_b, BQ, CK, lag, afirst):
    D, S = q_ref.shape if do_a else v_ref.shape
    c = (D ** -0.5) * LOG2E
    NQ, NK = S // BQ, S // CK
    st = {}

    def unit_a(u):
        j, ck = divmod(u, NK)
        cs = pl.ds(j * BQ, BQ)
        rs = pl.ds(ck * CK, CK)
        if ck == 0:
            st["q"] = (q_ref[:, cs].astype(jnp.float32) * c).astype(jnp.bfloat16)
            st["mx"] = None
        sT = lax.dot_general(k_ref[:, rs], st["q"], (((0,), (0,)), ((), ())),
                             preferred_element_type=jnp.float32)
        s_scr[rs, cs] = sT
        mm = jnp.max(sT.reshape(CK // 8, 8, BQ), axis=0)
        st["mx"] = mm if st["mx"] is None else jnp.maximum(st["mx"], mm)
        if ck == NK - 1:
            m_scr[:, cs] = st["mx"]

    def unit_b(u):
        j, ck = divmod(u, NK)
        cs = pl.ds(j * BQ, BQ)
        rs = pl.ds(ck * CK, CK)
        if ck == 0:
            st["m"] = jnp.max(m_scr[:, cs], axis=0, keepdims=True)
        p = jnp.exp2(s_scr[rs, cs] - st["m"])
        lc = jnp.sum(p.reshape(CK // 8, 8, BQ), axis=0)
        ob = jnp.dot(v_ref[:, rs], p.astype(jnp.bfloat16), preferred_element_type=jnp.float32)
        sl = j % 2
        if ck == 0:
            o_scr[sl] = ob
            l_scr[sl] = lc
        elif ck < NK - 1:
            o_scr[sl] += ob
            l_scr[sl] += lc
        else:
            lt = jnp.sum(l_scr[sl] + lc, axis=0, keepdims=True)
            o_ref[:, cs] = ((o_scr[sl] + ob) / lt).astype(o_ref.dtype)

    N = NQ * NK
    if not (do_a and do_b):
        def f(i, carry):
            return carry
        for u in range(N):
            (unit_a if do_a else unit_b)(u)
        return
    for u in range(min(lag, N)):
        unit_b(u)
    for u in range(N):
        if afirst:
            unit_a(u)
        if u + lag < N:
            unit_b(u + lag)
        if not afirst:
            unit_a(u)


def make(BQ=512, CK=128, lag=1, afirst=False, vmem=100 * 2**20, flags=None):
    def kernel(q_hbm, k_hbm, v_hbm, o_hbm, q_buf, k_buf, v_buf, o_buf, sems, osem,
               s_scr, m_scr, o_scr, l_scr, *, NH):
        def in_copies(slot, hq, hv):
            return (pltpu.make_async_copy(q_hbm.at[hq], q_buf.at[slot], sems.at[0, slot]),
                    pltpu.make_async_copy(k_hbm.at[hq], k_buf.at[slot], sems.at[1, slot]),
                    pltpu.make_async_copy(v_hbm.at[hv], v_buf.at[slot], sems.at[2, slot]))

        def out_copy(slot, h):
            return pltpu.make_async_copy(o_buf.at[slot], o_hbm.at[h], osem.at[slot])

        def body(slot, do_a, do_b):
            _body(q_buf.at[slot], k_buf.at[slot], v_buf.at[slot], o_buf.at[slot],
                  s_scr, m_scr, o_scr, l_scr, do_a=do_a, do_b=do_b, BQ=BQ, CK=CK, lag=lag, afirst=afirst)

        for cp in in_copies(0, 0, 0):
            cp.start()
        for cp in in_copies(1, 1, 0):
            cp.start()
        for cp in in_copies(0, 0, 0):
            cp.wait()
        body(0, True, False)

        def step(t, carry):
            slot = t % 2
            for cp in in_copies(slot, t, t - 1):
                cp.wait()
            for cp in in_copies(1 - slot, jnp.minimum(t + 1, NH - 1), t):
                cp.start()

            @pl.when(t >= 3)
            def _():
                out_copy(slot, t - 3).wait()
            body(slot, True, True)
            out_copy(slot, t - 1).start()
            return carry
        lax.fori_loop(1, NH, step, 0)

        slot = NH % 2
        for cp in in_copies(slot, NH - 1, NH - 1):
            cp.wait()
        out_copy(slot, NH - 3).wait()
        body(slot, False, True)
        out_copy(slot, NH - 1).start()
        out_copy(1 - slot, NH - 2).wait()
        out_copy(slot, NH - 1).wait()

    def fn(q, k, v):
        B, H, S, D = q.shape
        NH = B * H
        qT = jnp.swapaxes(q, 2, 3).reshape(NH, D, S)
        kT = jnp.swapaxes(k, 2, 3).reshape(NH, D, S)
        vT = jnp.swapaxes(v, 2, 3).reshape(NH, D, S)
        any_spec = pl.BlockSpec(memory_space=pl.ANY)
        buf = pltpu.VMEM((2, D, S), q.dtype)
        oT = pl.pallas_call(
            functools.partial(kernel, NH=NH),
            in_specs=[any_spec] * 3,
            out_specs=any_spec,
            out_shape=jax.ShapeDtypeStruct((NH, D, S), q.dtype),
            scratch_shapes=[buf, buf, buf, buf, pltpu.SemaphoreType.DMA((3, 2)), pltpu.SemaphoreType.DMA((2,)),
                            pltpu.VMEM((S, S), jnp.float32), pltpu.VMEM((8, S), jnp.float32),
                            pltpu.VMEM((2, D, BQ), jnp.float32), pltpu.VMEM((2, 8, BQ), jnp.float32)],
            compiler_params=pltpu.CompilerParams(vmem_limit_bytes=vmem,
                **({"flags": flags} if flags else {})),
            name="attn",
        )(qT, kT, vT)
        return jnp.swapaxes(oT.reshape(B, H, D, S), 2, 3)
    return fn


_impl = make(**dict())


@jax.jit
def pallas_standalone__fused_io_aware_attn__prompt_kernel(q, k, v):
    return _impl(q, k, v)
```
